```python
import os as _os
_os.environ.setdefault("JAX_PLATFORMS", "cpu")
import jax
import jax.numpy as jnp

def _softmax(x, axis=-1):
    return jax.nn.softmax(x, axis=axis)
def _gelu(x):
    return jax.nn.gelu(x, approximate=True)
def _silu(x):
    return jax.nn.silu(x)
def _sigmoid(x):
    return jax.nn.sigmoid(x)
def _layernorm(x, axis=-1, eps=1e-5):
    m = jnp.mean(x, axis=axis, keepdims=True)
    v = jnp.var(x, axis=axis, keepdims=True)
    return (x - m) / jnp.sqrt(v + eps)
def _scatter_add(tgt, idx, src, axis=0):
    return tgt.at[idx].add(src)
def _segment_sum(src, seg, n):
    return jax.ops.segment_sum(src, seg, n)
class _Rng:
    def __init__(self, key):
        self._k = key
    def _next(self):
        self._k, sub = jax.random.split(self._k)
        return sub
    def normal(self, shape):
        return jax.random.normal(self._next(), shape, dtype=jnp.bfloat16)
    def randint(self, lo, hi, shape):
        return jax.random.randint(self._next(), shape, lo, hi, dtype=jnp.int32)
    def uniform(self, shape, lo=0.0, hi=1.0):
        return jax.random.uniform(self._next(), shape, jnp.bfloat16, lo, hi)
    def permutation(self, n):
        return jax.random.permutation(self._next(), n)


kernel_name = 'interleave_layers__mha_block__dense_activation_mish__prompt'

def setup_inputs():
    _rng = _Rng(jax.random.key(int.from_bytes(__import__("os").urandom(4), "little")))
    _w = (lambda a: (lambda t: t.astype(jnp.bfloat16) if jnp.issubdtype(t.dtype, jnp.floating) else t)(jnp.asarray(a)))
    def _A_setup():
        B, S, D, H = 1, 2048, 512, 32
        return {
            "x": _w((lambda *s: _rng.normal(s) * 0.05)(B, S, D)),
            "wqkv": _w((lambda *s: _rng.normal(s) * 0.05)(D, 3 * D)),
            "wo": _w((lambda *s: _rng.normal(s) * 0.05)(D, D)),
        }
    _A_in = _A_setup()

    def _B_setup():
        B, S, D, F = 1, 2048, 512, 1792
        return {
            "x": _w((lambda *s: _rng.normal(s) * 0.05)(B, S, D)),
            "w1": _w((lambda *s: _rng.normal(s) * 0.4)(D, F) * (D ** -0.5)),
            "b1": _w((lambda *s: _rng.normal(s) * 0.4)(F)),
            "w2": _w((lambda *s: _rng.normal(s) * 0.4)(F, D) * (F ** -0.5)),
        }
    _B_in = _B_setup()

    return {
        "A_x": _A_in["x"],
        "A_wqkv": _A_in["wqkv"],
        "A_wo": _A_in["wo"],
        "B_x": _B_in["x"],
        "B_w1": _B_in["w1"],
        "B_b1": _B_in["b1"],
        "B_w2": _B_in["w2"],
    }

def reference(A_x, A_wqkv, A_wo, B_x, B_w1, B_b1, B_w2):
    def _A_ref(x, wqkv, wo):
        B, S, D = x.shape
        H = 32
        Dh = D // H
        qkv = (lambda x, *d: x.transpose(*d))((x @ wqkv).reshape(B, S, 3, H, Dh), 2, 0, 3, 1, 4)
        q, k, v = qkv[0], qkv[1], qkv[2]
        scores = jnp.einsum("bhqd,bhkd->bhqk", q, k) * (Dh ** -0.5)
        p = _softmax(scores, axis=-1)
        o = jnp.einsum("bhqk,bhkd->bhqd", p, v)
        return (lambda x, *d: x.transpose(*d))(o, 0, 2, 1, 3).reshape(B, S, D) @ wo

    def _B_ref(x, w1, b1, w2):
        h = jnp.einsum("bsd,df->bsf", x, w1) + b1
        sp = jnp.log1p(jnp.exp(-jnp.abs(h))) + jnp.where(h > 0, h, jnp.zeros_like(h))
        act = h * jnp.tanh(sp)
        return jnp.einsum("bsf,fd->bsd", act, w2)

    x = A_x
    x = x + _A_ref(_layernorm(x, axis=-1), A_wqkv, A_wo)
    x = x + _B_ref(_layernorm(x, axis=-1), B_w1, B_b1, B_w2)
    x = x + _A_ref(_layernorm(x, axis=-1), A_wqkv, A_wo)
    x = x + _B_ref(_layernorm(x, axis=-1), B_w1, B_b1, B_w2)
    return x
```

```python
import functools
import jax
import jax.numpy as jnp
from jax import lax
import jax.experimental.pallas as pl
import jax.experimental.pallas.tpu as pltpu

S, D, H, DH, F = 2048, 512, 32, 16, 1792
NG = D // 128
TQ = 512
NQ = S // TQ
TM = 256
EPS = 1e-5
LOG2E = 1.4426950408889634
NIT = H * NQ


def _ln(x):
    m = jnp.mean(x, axis=-1, keepdims=True)
    xc = x - m
    v = jnp.mean(xc * xc, axis=-1, keepdims=True)
    return xc * lax.rsqrt(v + EPS)


def _kernel(x_ref, wqkv_ref, wo_ref, w1_ref, b1_ref, w2_ref, o_ref,
            x_scr, wqT_scr, wvT_scr, k_scr, qT_scr, vT_scr, oT_scr, sA, sB, mA, mB):
    f32, bf16 = jnp.float32, jnp.bfloat16
    x_scr[...] = x_ref[...].astype(f32)
    vT_scr[:, DH:, :] = jnp.ones((H, DH, S), bf16)
    wqT_scr[...] = wqkv_ref[:, :D].astype(f32).T.astype(bf16)
    wvT_scr[...] = wqkv_ref[:, 2 * D:].astype(f32).T.astype(bf16)

    def qk_stage(i, s_ref, m_ref):
        h = i // NQ
        t = i % NQ
        g = h // 8
        j = h % 8
        rowid = lax.broadcasted_iota(jnp.int32, (128, TQ), 0) // DH
        qblk = qT_scr[t, pl.ds(pl.multiple_of(g * 128, 128), 128), :]
        qm = jnp.where(rowid == j, qblk, jnp.zeros_like(qblk))
        s = jnp.dot(k_scr[g], qm, preferred_element_type=f32)
        s_ref[...] = s
        m_ref[...] = jnp.max(s, axis=0, keepdims=True)

    def pv_stage(i, s_ref, m_ref):
        h = i // NQ
        t = i % NQ
        p = jnp.exp2(s_ref[...] - m_ref[...]).astype(bf16)
        o = jnp.dot(vT_scr[h], p, preferred_element_type=f32)
        on = o[:DH] / o[DH:DH + 1]
        oT_scr[t, pl.ds(pl.multiple_of(h * DH, DH), DH), :] = on.astype(bf16)

    def attention():
        for r in range(S // TM):
            rows = pl.ds(r * TM, TM)
            t = (r * TM) // TQ
            cols = pl.ds((r * TM) % TQ, TM)
            xn = _ln(x_scr[rows, :]).astype(bf16)
            k = jnp.dot(xn, wqkv_ref[:, D:2 * D], preferred_element_type=f32)
            for g in range(NG):
                k_scr[g, rows, :] = k[:, g * 128:(g + 1) * 128].astype(bf16)
            qT = lax.dot_general(wqT_scr[...], xn, (((1,), (1,)), ((), ())),
                                 preferred_element_type=f32)
            qT = (qT.astype(bf16).astype(f32) * (DH ** -0.5 * LOG2E)).astype(bf16)
            qT_scr[t, :, cols] = qT
            vT = lax.dot_general(wvT_scr[...], xn, (((1,), (1,)), ((), ())),
                                 preferred_element_type=f32)
            vT_scr[:, :DH, rows] = vT.astype(bf16).reshape(H, DH, TM)

        qk_stage(0, sA, mA)

        def body(jj, carry):
            i0 = 2 * jj
            qk_stage(i0 + 1, sB, mB)
            pv_stage(i0, sA, mA)
            qk_stage(jnp.minimum(i0 + 2, NIT - 1), sA, mA)
            pv_stage(i0 + 1, sB, mB)
            return carry
        lax.fori_loop(0, NIT // 2, body, 0)

        for r in range(S // TM):
            rows = pl.ds(r * TM, TM)
            t = (r * TM) // TQ
            cols = pl.ds((r * TM) % TQ, TM)
            out = lax.dot_general(oT_scr[t, :, cols], wo_ref[...], (((0,), (0,)), ((), ())),
                                  preferred_element_type=f32)
            x_scr[rows, :] += out

    def mlp():
        for r in range(S // TM):
            rows = pl.ds(r * TM, TM)
            x = x_scr[rows, :]
            xn = _ln(x).astype(bf16)
            hh = jnp.dot(xn, w1_ref[...], preferred_element_type=f32) + b1_ref[...].astype(f32)
            sp = jnp.log1p(jnp.exp(-jnp.abs(hh))) + jnp.maximum(hh, 0.0)
            act = (hh * jnp.tanh(sp)).astype(bf16)
            x_scr[rows, :] = x + jnp.dot(act, w2_ref[...], preferred_element_type=f32)

    for _ in range(2):
        attention()
        mlp()
    o_ref[...] = x_scr[...].astype(o_ref.dtype)


@jax.jit
def pallas_interleave_layers__mha_block__dense_activation_mish__prompt_kernel(A_x, A_wqkv, A_wo, B_x, B_w1, B_b1, B_w2):
    x = A_x.reshape(S, D)
    b1 = B_b1.reshape(1, F)
    out = pl.pallas_call(
        _kernel,
        out_shape=jax.ShapeDtypeStruct((S, D), jnp.bfloat16),
        scratch_shapes=[
            pltpu.VMEM((S, D), jnp.float32),
            pltpu.VMEM((D, D), jnp.bfloat16),
            pltpu.VMEM((D, D), jnp.bfloat16),
            pltpu.VMEM((NG, S, 128), jnp.bfloat16),
            pltpu.VMEM((NQ, D, TQ), jnp.bfloat16),
            pltpu.VMEM((H, 2 * DH, S), jnp.bfloat16),
            pltpu.VMEM((NQ, D, TQ), jnp.bfloat16),
            pltpu.VMEM((S, TQ), jnp.float32),
            pltpu.VMEM((S, TQ), jnp.float32),
            pltpu.VMEM((1, TQ), jnp.float32),
            pltpu.VMEM((1, TQ), jnp.float32),
        ],
        compiler_params=pltpu.CompilerParams(vmem_limit_bytes=100 * 1024 * 1024),
    )(x, A_wqkv, A_wo, B_w1, b1, B_w2)
    return out.reshape(1, S, D)
```

```python
import functools
import jax
import jax.numpy as jnp
from jax import lax
import jax.experimental.pallas as pl
import jax.experimental.pallas.tpu as pltpu

S, D, H, DH, F = 2048, 512, 32, 16, 1792
TQ = 512
NQ = S // TQ
CK = 128
NC = S // CK
LAG = 2
THR = 4
TM = 256
EPS = 1e-5
LOG2E = 1.4426950408889634
NIT = H * NQ


def _ln(x):
    m = jnp.mean(x, axis=-1, keepdims=True)
    xc = x - m
    v = jnp.mean(xc * xc, axis=-1, keepdims=True)
    return xc * lax.rsqrt(v + EPS)


def _kernel(x_ref, wqkv_ref, wo_hbm, w1_hbm, b1_ref, w2_hbm, o_hbm,
            x_scr, wqT_scr, wvT_scr, k_scr, qT_scr, vT_scr, oT_scr, sA, sB, mA, mB, xA, xB,
            wo_ref, w1_ref, w2_ref, o_stage, w_sems, o_sems):
    f32, bf16 = jnp.float32, jnp.bfloat16
    w_copies = [pltpu.make_async_copy(src_, dst_, w_sems.at[n])
                for n, (src_, dst_) in enumerate(((wo_hbm, wo_ref), (w1_hbm, w1_ref), (w2_hbm, w2_ref)))]
    for cp in w_copies:
        cp.start()
    o_copies = [pltpu.make_async_copy(o_stage.at[pl.ds(r * TM, TM)], o_hbm.at[pl.ds(r * TM, TM)], o_sems.at[r])
                for r in range(S // TM)]
    x_scr[...] = x_ref[...].astype(f32)
    wqT_scr[...] = wqkv_ref[:, :D].astype(f32).T.astype(bf16)
    wvT_scr[...] = wqkv_ref[:, 2 * D:].astype(f32).T.astype(bf16)

    def qblk_of(i):
        h = i // NQ
        t = i % NQ
        return h, qT_scr[t, pl.ds(pl.multiple_of(h * DH, DH), DH), :]

    def qk_chunk(h, qblk, c, s_ref, mx):
        rows = pl.ds(c * CK, CK)
        s = jnp.dot(k_scr[h, rows, :], qblk, preferred_element_type=f32)
        s_ref[rows, :] = s
        return jnp.maximum(mx, jnp.max(s.reshape(CK // 8, 8, TQ), axis=0))

    def stage(i, X, mX, xX, Y, mY, xY, do1=True, do2=True):
        if do1:
            h1, q1 = qblk_of(i + 1)
            mxY = xY[...]
        if do2:
            h2, q2 = qblk_of(i + 2)
            mxX = jnp.full((8, TQ), -jnp.inf, f32)
        hp = i // NQ
        tp = i % NQ
        mp = mX[...]
        acc = jnp.zeros((DH, TQ), f32)
        lsum = jnp.zeros((8, TQ), f32)
        accs = []
        for c in range(NC):
            if c + LAG < NC:
                if do1:
                    mxY = qk_chunk(h1, q1, c + LAG, Y, mxY)
                    if c + LAG == NC - 1:
                        mY[...] = jnp.max(mxY, axis=0, keepdims=True)
            elif do2:
                mxX = qk_chunk(h2, q2, c + LAG - NC, X, mxX)
            rows = pl.ds(c * CK, CK)
            if c >= THR:
                dep = accs[c - THR][0:1]
                mpc = mp + (dep - dep)
            else:
                mpc = mp
            p32 = jnp.exp2(X[rows, :] - mpc)
            lsum = lsum + jnp.sum(p32.reshape(CK // 8, 8, TQ), axis=0)
            acc = acc + jnp.dot(vT_scr[hp, :, rows], p32.astype(bf16), preferred_element_type=f32)
            accs.append(acc)
        if do2:
            xX[...] = mxX
        on = acc / jnp.sum(lsum, axis=0, keepdims=True)
        oT_scr[tp, pl.ds(pl.multiple_of(hp * DH, DH), DH), :] = on.astype(bf16)

    def attention(first):
        for r in range(S // TM):
            rows = pl.ds(r * TM, TM)
            t = (r * TM) // TQ
            cols = pl.ds((r * TM) % TQ, TM)
            xn = _ln(x_scr[rows, :]).astype(bf16)
            k = jnp.dot(xn, wqkv_ref[:, D:2 * D], preferred_element_type=f32).astype(bf16)
            for h in range(H):
                k_scr[h, rows, :] = k[:, h * DH:(h + 1) * DH]
            qT = lax.dot_general(wqT_scr[...], xn, (((1,), (1,)), ((), ())),
                                 preferred_element_type=f32)
            qT = (qT.astype(bf16).astype(f32) * (DH ** -0.5 * LOG2E)).astype(bf16)
            qT_scr[t, :, cols] = qT
            vT = lax.dot_general(wvT_scr[...], xn, (((1,), (1,)), ((), ())),
                                 preferred_element_type=f32)
            vT_scr[:, :, rows] = vT.astype(bf16).reshape(H, DH, TM)

        h0, q0 = qblk_of(0)
        mx = jnp.full((8, TQ), -jnp.inf, f32)
        for c in range(NC):
            mx = qk_chunk(h0, q0, c, sA, mx)
        mA[...] = jnp.max(mx, axis=0, keepdims=True)
        h1, q1 = qblk_of(1)
        mx = jnp.full((8, TQ), -jnp.inf, f32)
        for c in range(LAG):
            mx = qk_chunk(h1, q1, c, sB, mx)
        xB[...] = mx

        def body(jj, carry):
            i0 = 2 * jj
            stage(i0, sA, mA, xA, sB, mB, xB)
            stage(i0 + 1, sB, mB, xB, sA, mA, xA)
            return carry
        lax.fori_loop(0, NIT // 2 - 1, body, 0)
        stage(NIT - 2, sA, mA, xA, sB, mB, xB, do2=False)
        stage(NIT - 1, sB, mB, xB, sA, mA, xA, do1=False, do2=False)

        if first:
            for cp in w_copies:
                cp.wait()

        for r in range(S // TM):
            rows = pl.ds(r * TM, TM)
            t = (r * TM) // TQ
            cols = pl.ds((r * TM) % TQ, TM)
            out = lax.dot_general(oT_scr[t, :, cols], wo_ref[...], (((0,), (0,)), ((), ())),
                                  preferred_element_type=f32)
            x_scr[rows, :] += out

    def mlp(last):
        for r in range(S // TM):
            rows = pl.ds(r * TM, TM)
            x = x_scr[rows, :]
            xn = _ln(x).astype(bf16)
            hh = jnp.dot(xn, w1_ref[...], preferred_element_type=f32) + b1_ref[...].astype(f32)
            sp = jnp.log1p(jnp.exp(-jnp.abs(hh))) + jnp.maximum(hh, 0.0)
            act = (hh * jnp.tanh(sp)).astype(bf16)
            y = x + jnp.dot(act, w2_ref[...], preferred_element_type=f32)
            if last:
                o_stage[rows, :] = y.astype(bf16)
                o_copies[r].start()
            else:
                x_scr[rows, :] = y

    for layer in range(2):
        attention(layer == 0)
        mlp(layer == 1)
    for cp in o_copies:
        cp.wait()


@jax.jit
def pallas_interleave_layers__mha_block__dense_activation_mish__prompt_kernel(A_x, A_wqkv, A_wo, B_x, B_w1, B_b1, B_w2):
    x = A_x.reshape(S, D)
    b1 = B_b1.reshape(1, F)
    out = pl.pallas_call(
        _kernel,
        out_shape=jax.ShapeDtypeStruct((S, D), jnp.bfloat16),
        in_specs=[
            pl.BlockSpec(memory_space=pltpu.VMEM),
            pl.BlockSpec(memory_space=pltpu.VMEM),
            pl.BlockSpec(memory_space=pl.ANY),
            pl.BlockSpec(memory_space=pl.ANY),
            pl.BlockSpec(memory_space=pltpu.VMEM),
            pl.BlockSpec(memory_space=pl.ANY),
        ],
        out_specs=pl.BlockSpec(memory_space=pl.ANY),
        scratch_shapes=[
            pltpu.VMEM((S, D), jnp.float32),
            pltpu.VMEM((D, D), jnp.bfloat16),
            pltpu.VMEM((D, D), jnp.bfloat16),
            pltpu.VMEM((H, S, DH), jnp.bfloat16),
            pltpu.VMEM((NQ, D, TQ), jnp.bfloat16),
            pltpu.VMEM((H, DH, S), jnp.bfloat16),
            pltpu.VMEM((NQ, D, TQ), jnp.bfloat16),
            pltpu.VMEM((S, TQ), jnp.float32),
            pltpu.VMEM((S, TQ), jnp.float32),
            pltpu.VMEM((1, TQ), jnp.float32),
            pltpu.VMEM((1, TQ), jnp.float32),
            pltpu.VMEM((8, TQ), jnp.float32),
            pltpu.VMEM((8, TQ), jnp.float32),
            pltpu.VMEM((D, D), jnp.bfloat16),
            pltpu.VMEM((D, F), jnp.bfloat16),
            pltpu.VMEM((F, D), jnp.bfloat16),
            pltpu.VMEM((S, D), jnp.bfloat16),
            pltpu.SemaphoreType.DMA((3,)),
            pltpu.SemaphoreType.DMA((S // TM,)),
        ],
        compiler_params=pltpu.CompilerParams(vmem_limit_bytes=100 * 1024 * 1024),
    )(x, A_wqkv, A_wo, B_w1, b1, B_w2)
    return out.reshape(1, S, D)
```

```python
import jax
import jax.numpy as jnp
from jax import lax
import jax.experimental.pallas as pl
import jax.experimental.pallas.tpu as pltpu

S, D, H, DH, F = 2048, 512, 32, 16, 1792
TQ = 512
NQ = S // TQ
CK = 128
NC = S // CK
LAG = 1
THR = 4
TM = 256
EPS = 1e-5
LOG2E = 1.4426950408889634


def _ln(x):
    m = jnp.mean(x, axis=-1, keepdims=True)
    xc = x - m
    v = jnp.mean(xc * xc, axis=-1, keepdims=True)
    return xc * lax.rsqrt(v + EPS)


def _kernel(x_ref, wqkv_ref, wo_hbm, w1_hbm, b1_ref, w2_hbm, o_hbm,
            x_scr, wqT_scr, wvT_scr, k_scr, qT_scr, vT_scr, oT_scr, sA, sB, mA, mB, xA, xB,
            wo_ref, w1_ref, w2_ref, o_stage, w_sems, o_sems):
    f32, bf16 = jnp.float32, jnp.bfloat16
    w_copies = [pltpu.make_async_copy(src_, dst_, w_sems.at[n])
                for n, (src_, dst_) in enumerate(((wo_hbm, wo_ref), (w1_hbm, w1_ref), (w2_hbm, w2_ref)))]
    for cp in w_copies:
        cp.start()
    o_copies = [pltpu.make_async_copy(o_stage.at[pl.ds(r * TM, TM)], o_hbm.at[pl.ds(r * TM, TM)], o_sems.at[r])
                for r in range(S // TM)]
    x_scr[...] = x_ref[...].astype(f32)
    wqT_scr[...] = wqkv_ref[:, :D].astype(f32).T.astype(bf16)
    wvT_scr[...] = wqkv_ref[:, 2 * D:].astype(f32).T.astype(bf16)

    def qblk_of(h, t):
        h = h + t // NQ
        t = t % NQ
        return h, qT_scr[t, pl.ds(pl.multiple_of(h * DH, DH), DH), :]

    def qk_chunk(h, qblk, c, s_ref, mx):
        rows = pl.ds(c * CK, CK)
        s = jnp.dot(k_scr[h, rows, :], qblk, preferred_element_type=f32)
        s_ref[rows, :] = s
        return jnp.maximum(mx, jnp.max(s.reshape(CK // 8, 8, TQ), axis=0))

    def stage(hp, tp, X, mX, xX, Y, mY, xY, do1=True, do2=True):
        if do1:
            h1, q1 = qblk_of(hp, tp + 1)
            mxY = xY[...]
        if do2:
            h2, q2 = qblk_of(hp, tp + 2)
            mxX = jnp.full((8, TQ), -jnp.inf, f32)
        mp = mX[...]
        acc = jnp.zeros((DH, TQ), f32)
        lsum = jnp.zeros((8, TQ), f32)
        accs = []
        for c in range(NC):
            if c + LAG < NC:
                if do1:
                    mxY = qk_chunk(h1, q1, c + LAG, Y, mxY)
                    if c + LAG == NC - 1:
                        mY[...] = jnp.max(mxY, axis=0, keepdims=True)
            elif do2:
                mxX = qk_chunk(h2, q2, c + LAG - NC, X, mxX)
            rows = pl.ds(c * CK, CK)
            if c >= THR:
                dep = accs[c - THR][0:1]
                mpc = mp + (dep - dep)
            else:
                mpc = mp
            p32 = jnp.exp2(X[rows, :] - mpc)
            lsum = lsum + jnp.sum(p32.reshape(CK // 8, 8, TQ), axis=0)
            acc = acc + jnp.dot(vT_scr[hp, :, rows], p32.astype(bf16), preferred_element_type=f32)
            accs.append(acc)
        if do2:
            xX[...] = mxX
        on = acc / jnp.sum(lsum, axis=0, keepdims=True)
        oT_scr[tp, pl.ds(pl.multiple_of(hp * DH, DH), DH), :] = on.astype(bf16)

    def attention(first):
        for r in range(S // TM):
            rows = pl.ds(r * TM, TM)
            t = (r * TM) // TQ
            cols = pl.ds((r * TM) % TQ, TM)
            xn = _ln(x_scr[rows, :]).astype(bf16)
            k = jnp.dot(xn, wqkv_ref[:, D:2 * D], preferred_element_type=f32).astype(bf16)
            for h in range(H):
                k_scr[h, rows, :] = k[:, h * DH:(h + 1) * DH]
            qT = lax.dot_general(wqT_scr[...], xn, (((1,), (1,)), ((), ())),
                                 preferred_element_type=f32)
            qT = (qT.astype(bf16).astype(f32) * (DH ** -0.5 * LOG2E)).astype(bf16)
            qT_scr[t, :, cols] = qT
            vT = lax.dot_general(wvT_scr[...], xn, (((1,), (1,)), ((), ())),
                                 preferred_element_type=f32)
            vT_scr[:, :, rows] = vT.astype(bf16).reshape(H, DH, TM)

        h0, q0 = qblk_of(0, 0)
        mx = jnp.full((8, TQ), -jnp.inf, f32)
        for c in range(NC):
            mx = qk_chunk(h0, q0, c, sA, mx)
        mA[...] = jnp.max(mx, axis=0, keepdims=True)
        h1, q1 = qblk_of(0, 1)
        mx = jnp.full((8, TQ), -jnp.inf, f32)
        for c in range(LAG):
            mx = qk_chunk(h1, q1, c, sB, mx)
        xB[...] = mx

        def body(h, carry):
            stage(h, 0, sA, mA, xA, sB, mB, xB)
            stage(h, 1, sB, mB, xB, sA, mA, xA)
            stage(h, 2, sA, mA, xA, sB, mB, xB)
            stage(h, 3, sB, mB, xB, sA, mA, xA)
            return carry
        lax.fori_loop(0, H - 1, body, 0)
        stage(H - 1, 0, sA, mA, xA, sB, mB, xB)
        stage(H - 1, 1, sB, mB, xB, sA, mA, xA)
        stage(H - 1, 2, sA, mA, xA, sB, mB, xB, do2=False)
        stage(H - 1, 3, sB, mB, xB, sA, mA, xA, do1=False, do2=False)

        if first:
            for cp in w_copies:
                cp.wait()

        for r in range(S // TM):
            rows = pl.ds(r * TM, TM)
            t = (r * TM) // TQ
            cols = pl.ds((r * TM) % TQ, TM)
            out = lax.dot_general(oT_scr[t, :, cols], wo_ref[...], (((0,), (0,)), ((), ())),
                                  preferred_element_type=f32)
            x_scr[rows, :] += out

    def mlp(last):
        for r in range(S // TM):
            rows = pl.ds(r * TM, TM)
            x = x_scr[rows, :]
            xn = _ln(x).astype(bf16)
            hh = jnp.dot(xn, w1_ref[...], preferred_element_type=f32) + b1_ref[...].astype(f32).reshape(1, F)
            sp = jnp.log1p(jnp.exp(-jnp.abs(hh))) + jnp.maximum(hh, 0.0)
            act = (hh * jnp.tanh(sp)).astype(bf16)
            y = x + jnp.dot(act, w2_ref[...], preferred_element_type=f32)
            if last:
                o_stage[rows, :] = y.astype(bf16)
                o_copies[r].start()
            else:
                x_scr[rows, :] = y

    for layer in range(2):
        attention(layer == 0)
        mlp(layer == 1)
    for cp in o_copies:
        cp.wait()


@jax.jit
def pallas_interleave_layers__mha_block__dense_activation_mish__prompt_kernel(
    A_x: jax.Array,
    A_wqkv: jax.Array,
    A_wo: jax.Array,
    B_x: jax.Array,
    B_w1: jax.Array,
    B_b1: jax.Array,
    B_w2: jax.Array,
):
    x = A_x.reshape(S, D)
    out = pl.pallas_call(
        _kernel,
        out_shape=jax.ShapeDtypeStruct((S, D), jnp.bfloat16),
        in_specs=[
            pl.BlockSpec(memory_space=pltpu.VMEM),
            pl.BlockSpec(memory_space=pltpu.VMEM),
            pl.BlockSpec(memory_space=pl.ANY),
            pl.BlockSpec(memory_space=pl.ANY),
            pl.BlockSpec(memory_space=pltpu.VMEM),
            pl.BlockSpec(memory_space=pl.ANY),
        ],
        out_specs=pl.BlockSpec(memory_space=pl.ANY),
        scratch_shapes=[
            pltpu.VMEM((S, D), jnp.float32),
            pltpu.VMEM((D, D), jnp.bfloat16),
            pltpu.VMEM((D, D), jnp.bfloat16),
            pltpu.VMEM((H, S, DH), jnp.bfloat16),
            pltpu.VMEM((NQ, D, TQ), jnp.bfloat16),
            pltpu.VMEM((H, DH, S), jnp.bfloat16),
            pltpu.VMEM((NQ, D, TQ), jnp.bfloat16),
            pltpu.VMEM((S, TQ), jnp.float32),
            pltpu.VMEM((S, TQ), jnp.float32),
            pltpu.VMEM((1, TQ), jnp.float32),
            pltpu.VMEM((1, TQ), jnp.float32),
            pltpu.VMEM((8, TQ), jnp.float32),
            pltpu.VMEM((8, TQ), jnp.float32),
            pltpu.VMEM((D, D), jnp.bfloat16),
            pltpu.VMEM((D, F), jnp.bfloat16),
            pltpu.VMEM((F, D), jnp.bfloat16),
            pltpu.VMEM((S, D), jnp.bfloat16),
            pltpu.SemaphoreType.DMA((3,)),
            pltpu.SemaphoreType.DMA((S // TM,)),
        ],
        compiler_params=pltpu.CompilerParams(vmem_limit_bytes=100 * 1024 * 1024),
    )(x, A_wqkv, A_wo, B_w1, B_b1, B_w2)
    return out.reshape(1, S, D)
```
